```python
import jax
import jax.numpy as jnp

def _softmax(x, axis=-1):
    return jax.nn.softmax(x, axis=axis)
def _gelu(x):
    return jax.nn.gelu(x, approximate=True)
def _silu(x):
    return jax.nn.silu(x)
def _sigmoid(x):
    return jax.nn.sigmoid(x)
def _layernorm(x, axis=-1, eps=1e-5):
    m = jnp.mean(x, axis=axis, keepdims=True)
    v = jnp.var(x, axis=axis, keepdims=True)
    return (x - m) / jnp.sqrt(v + eps)
def _scatter_add(tgt, idx, src, axis=0):
    return tgt.at[idx].add(src)
def _segment_sum(src, seg, n):
    return jax.ops.segment_sum(src, seg, n)
class _Rng:
    def __init__(self, key):
        self._k = key
    def _next(self):
        self._k, sub = jax.random.split(self._k)
        return sub
    def normal(self, shape):
        return jax.random.normal(self._next(), shape, dtype=jnp.bfloat16)
    def randint(self, lo, hi, shape):
        return jax.random.randint(self._next(), shape, lo, hi, dtype=jnp.int32)
    def uniform(self, shape, lo=0.0, hi=1.0):
        return jax.random.uniform(self._next(), shape, jnp.bfloat16, lo, hi)
    def permutation(self, n):
        return jax.random.permutation(self._next(), n)


kernel_name = 'recurrent_scan__linear_kernel_hedgehog__dense_activation_relu__prompt'

def _fwd_setup_inputs():
    _rng = _Rng(jax.random.key(int.from_bytes(__import__("os").urandom(4), "little")))
    _w = (lambda a: (lambda t: t.astype(jnp.bfloat16) if jnp.issubdtype(t.dtype, jnp.floating) else t)(jnp.asarray(a)))
    def _A_setup():
        B, S, D, H = 1, 2048, 1024, 32
        Dh = D // H
        return {
            "x": _w((lambda *s: _rng.normal(s) * 0.05)(B, S, D)),
            "wqkv": _w((lambda *s: _rng.normal(s) * 0.05)(D, 3 * D)),
            "w_phi": _w((lambda *s: _rng.normal(s) * 0.05)(H, Dh, Dh) * (Dh ** -0.5)),
            "wo": _w((lambda *s: _rng.normal(s) * 0.05)(D, D)),
        }
    _A_in = _A_setup()

    def _B_setup():
        B, S, D, Dff = 1, 2048, 1024, 3584
        return {
            "x": _w((lambda *s: _rng.normal(s) * 0.05)(B, S, D)),
            "w1": _w((lambda *s: _rng.normal(s) * 0.05)(D, Dff)),
            "w2": _w((lambda *s: _rng.normal(s) * 0.05)(Dff, D)),
        }
    _B_in = _B_setup()

    return {
        "A_x": _A_in["x"],
        "A_wqkv": _A_in["wqkv"],
        "A_w_phi": _A_in["w_phi"],
        "A_wo": _A_in["wo"],
        "B_x": _B_in["x"],
        "B_w1": _B_in["w1"],
        "B_w2": _B_in["w2"],
    }

def _fwd_reference(A_x, A_wqkv, A_w_phi, A_wo, B_x, B_w1, B_w2):
    def _A_ref(x, wqkv, w_phi, wo):
        B, S, D = x.shape
        H = 32; Dh = D // H
        qkv = (lambda x, *d: x.transpose(*d))((x @ wqkv).reshape(B, S, 3, H, Dh), 2, 0, 3, 1, 4)
        q, k, v = qkv[0], qkv[1], qkv[2]
        pq = jnp.einsum("bhsd,hdf->bhsf", q, w_phi)
        pk = jnp.einsum("bhsd,hdf->bhsf", k, w_phi)
        phi_q = jnp.concatenate([_softmax(pq, axis=-1), _softmax(-pq, axis=-1)], axis=-1)
        phi_k = jnp.concatenate([_softmax(pk, axis=-1), _softmax(-pk, axis=-1)], axis=-1)
        kv = jnp.einsum("bhsf,bhsd->bhfd", phi_k, v)
        z  = jnp.einsum("bhsf->bhf", phi_k)
        num = jnp.einsum("bhqf,bhfd->bhqd", phi_q, kv)
        den = jnp.einsum("bhqf,bhf->bhq", phi_q, z)[..., None] + 1e-6
        o = num / den
        return (lambda x, *d: x.transpose(*d))(o, 0, 2, 1, 3).reshape(B, S, D) @ wo

    def _B_ref(x, w1, w2):
        h = jnp.einsum("bsd,df->bsf", x, w1)
        zero = jnp.zeros_like(h)
        h = jnp.maximum(h, zero)
        return jnp.einsum("bsf,fd->bsd", h, w2)

    x = A_x
    xn = _layernorm(x, axis=-1)
    s = _A_ref(xn, A_wqkv, A_w_phi, A_wo)
    g = _silu(_B_ref(xn, B_w1, B_w2))
    return x + s * g


def setup_inputs():
    _inp = _fwd_setup_inputs()
    _gk = jax.random.fold_in(jax.random.key(int.from_bytes(__import__("os").urandom(4), "little")), 2**31 - 1)
    _shapes = [[1, 2048, 1024]]
    _dtypes = ['bfloat16']
    _gks = jax.random.split(_gk, len(_shapes))
    _gs = [jax.random.normal(k, s, dtype=jnp.dtype(d)) * 0.05 for k, s, d in zip(_gks, _shapes, _dtypes)]
    _inp["grad_out"] = _gs[0]
    return _inp

def reference(A_x, A_wqkv, A_w_phi, A_wo, B_w1, B_w2, B_x, grad_out):
    _const = dict(B_x=B_x)
    def _f(*_d):
        return _fwd_reference(**{'A_x': _d[0], 'A_wqkv': _d[1], 'A_w_phi': _d[2], 'A_wo': _d[3], 'B_w1': _d[4], 'B_w2': _d[5], **_const})
    _out, _vjp = jax.vjp(_f, A_x, A_wqkv, A_w_phi, A_wo, B_w1, B_w2)
    _grads = _vjp(grad_out)
    _out0 = jnp.asarray(_out)
    return (_out0, *[jnp.asarray(_g) for _g in _grads])
```

```python
import jax
import jax.numpy as jnp
from jax import lax
import jax.experimental.pallas as pl
import jax.experimental.pallas.tpu as pltpu

S, D, H, DH, F = 2048, 1024, 32, 32, 3584
T = 256
NT = S // T
FC = 512
NF = F // FC
G = D // 128
BF, F32 = jnp.bfloat16, jnp.float32


def _nn(a, b):
    return lax.dot_general(a, b, (((1,), (0,)), ((), ())), preferred_element_type=F32)


def _nt(a, b):
    return lax.dot_general(a, b, (((1,), (1,)), ((), ())), preferred_element_type=F32)


def _tn(a, b):
    return lax.dot_general(a, b, (((0,), (0,)), ((), ())), preferred_element_type=F32)


def _head_mask(rows):
    r = lax.broadcasted_iota(jnp.int32, (rows, 128), 0)
    c = lax.broadcasted_iota(jnp.int32, (rows, 128), 1)
    return ((r >> 5) & 3) == (c >> 5)


def _heads(x):
    return x.reshape(x.shape[0] // DH, DH, x.shape[1])


def _flat(x):
    return x.reshape(x.shape[0] * DH, x.shape[2])


def _dual_softmax(p):
    p3 = _heads(p)
    ep = jnp.exp(p3 - jnp.max(p3, axis=1, keepdims=True))
    em = jnp.exp(jnp.min(p3, axis=1, keepdims=True) - p3)
    fp = ep * (1.0 / jnp.sum(ep, axis=1, keepdims=True))
    fm = em * (1.0 / jnp.sum(em, axis=1, keepdims=True))
    return _flat(fp), _flat(fm)


def _dual_softmax_bwd(fp, fm, dfp, dfm):
    fp, fm, dfp, dfm = _heads(fp), _heads(fm), _heads(dfp), _heads(dfm)
    a = fp * (dfp - jnp.sum(fp * dfp, axis=1, keepdims=True))
    b = fm * (dfm - jnp.sum(fm * dfm, axis=1, keepdims=True))
    return _flat(a - b)


def _lane_fold(x):
    acc = x[:, 0:128]
    for j in range(1, x.shape[1] // 128):
        acc = acc + x[:, j * 128:(j + 1) * 128]
    return acc


def _lane_rep(x):
    return jnp.concatenate([x] * (T // 128), axis=1)


def _center(x):
    x3 = _heads(x)
    return _flat(x3 - jnp.mean(x3, axis=1, keepdims=True))


def _kernel(x_h, wqkv_h, wphi_ref, wo_h, w1_h, w2_h, go_h,
            out_h, dx_h, dwqkv_h, dwphi_ref, dwo_h, dw1_h, dw2_h,
            xb, gob, xnT, ab, dhb, dyT, qT, w1b, w2b, wT, wqk, wob, dwo_acc,
            bd, bdT, rstdT, acc, zacc, kvT, kvc, zb, zc, isem, osem):
    def cp(src, dst, sem):
        return pltpu.make_async_copy(src, dst, sem)

    in_x = cp(x_h, xb, isem.at[0])
    in_wq = cp(wqkv_h.at[:, 0:D], wqk.at[0], isem.at[1])
    in_wk = cp(wqkv_h.at[:, D:2 * D], wqk.at[1], isem.at[2])
    in_wv = cp(wqkv_h.at[:, 2 * D:3 * D], wT.at[0], isem.at[3])
    in_w1 = cp(w1_h, w1b, isem.at[4])
    in_w2 = cp(w2_h, w2b, isem.at[5])
    in_wo = cp(wo_h, wob, isem.at[6])
    in_go = cp(go_h, gob, isem.at[7])
    in_wk.start()
    in_wv.start()
    in_x.start()

    w = wphi_ref[...].astype(F32)
    wbd = jnp.where(_head_mask(D), jnp.concatenate([w] * 4, axis=1), 0.0)
    bd[...] = wbd.astype(BF)
    for g in range(G):
        bdT[g * 128:(g + 1) * 128, :] = wbd[g * 128:(g + 1) * 128, :].T.astype(BF)
    acc[...] = jnp.zeros(acc.shape, F32)
    zacc[...] = jnp.zeros(zacc.shape, F32)

    def fold_t(j):
        for g in range(G):
            r = slice(g * 128, (g + 1) * 128)
            wT[j, r, :] = _nt(bdT[r, :], wqk[j, :, r]).astype(BF)

    in_wk.wait()
    fold_t(1)
    in_wv.wait()
    in_w1.start()
    for g in range(G):
        r = slice(g * 128, (g + 1) * 128)
        wT[2, r, :] = wT[0, :, r].astype(F32).T.astype(BF)
    in_x.wait()
    in_w1.wait()
    in_wq.start()
    in_wo.start()
    in_w2.start()
    in_go.start()

    def p1(t, carry):
        tok = pl.ds(pl.multiple_of(t * T, T), T)
        x = xb[tok, :].astype(F32)
        xc = x - jnp.mean(x, axis=1, keepdims=True)
        rstd = lax.rsqrt(jnp.mean(xc * xc, axis=1, keepdims=True) + 1e-5)
        xn32 = xc * rstd
        xn = xn32.astype(BF)
        xnT[:, tok] = xn32.T.astype(BF)
        rstdT[:, tok] = jnp.broadcast_to(rstd, (T, 128)).T[0:8, :]
        pk = _nt(wT[1], xn)
        v = _nt(wT[2], xn).astype(BF)
        qT[2, :, tok] = v
        for c in range(NF):
            cs = slice(c * FC, (c + 1) * FC)
            h = _nn(xn, w1b[:, cs])
            ab[tok, cs] = jnp.where(h < 0.0, -0.0, jnp.abs(h)).astype(BF)
        for g in range(G):
            r = slice(g * 128, (g + 1) * 128)
            fp, fm = _dual_softmax(pk[r, :])
            ph = jnp.concatenate([fp, fm], axis=0)
            phb = ph.astype(BF)
            qT[1, r, tok] = phb[0:128]
            qT[3, r, tok] = phb[128:256]
            acc[g] += _nt(phb, v[r, :])
            zacc[g] += _lane_fold(ph)
        return carry

    lax.fori_loop(0, NT, p1, 0)

    def finish_state():
        m = _head_mask(256)
        for g in range(G):
            kv = jnp.where(m, acc[g], 0.0)
            kvT[g] = kv.T.astype(BF)
            kvc[g] = _center(kv).astype(BF)
            z = jnp.broadcast_to(jnp.sum(zacc[g], axis=1, keepdims=True), (256, 128))
            zb[g] = z
            zc[g] = _center(z)

    finish_state()
    acc[...] = jnp.zeros(acc.shape, F32)
    zacc[...] = jnp.zeros(zacc.shape, F32)
    dwo_acc[...] = jnp.zeros(dwo_acc.shape, F32)
    in_wq.wait()
    fold_t(0)
    in_wo.wait()
    in_w2.wait()
    in_go.wait()

    def p2(t, carry):
        tok = pl.ds(pl.multiple_of(t * T, T), T)
        pq = _nn(wT[0], xnT[:, tok])
        y = _nn(ab[tok, :], w2b[...])
        phis, outs, invs = [], [], []
        for g in range(G):
            r = slice(g * 128, (g + 1) * 128)
            fp, fm = _dual_softmax(pq[r, :])
            ph = jnp.concatenate([fp, fm], axis=0)
            pz = ph * _lane_rep(zb[g])
            den = jnp.sum(_heads(pz[0:128] + pz[128:256]), axis=1, keepdims=True) + 1e-6
            inv = 1.0 / den
            o = _flat(_heads(_nn(kvT[g], ph.astype(BF))) * inv)
            phis.append(ph)
            outs.append(o)
            invs.append(inv)
        oT = jnp.concatenate(outs, axis=0)
        s = _nn(oT.T.astype(BF), wob[...])
        sig = 1.0 / (1.0 + jnp.exp(-y))
        gate = y * sig
        go = gob[tok, :].astype(F32)
        xb[tok, :] = (xb[tok, :].astype(F32) + s * gate).astype(BF)
        cp(xb.at[tok], out_h.at[tok], osem.at[0, t]).start()
        ds = (go * gate).astype(BF)
        dy32 = go * s * (sig * (1.0 + y * (1.0 - sig)))
        dy = dy32.astype(BF)
        dyT[:, tok] = dy32.T.astype(BF)
        doT = _nt(wob[...], ds)
        dwo_acc[...] += _nn(oT.astype(BF), ds)
        for c in range(NF):
            cs = slice(c * FC, (c + 1) * FC)
            da = _nt(dy, w2b[cs, :])
            bits = lax.bitcast_convert_type(ab[tok, cs].astype(F32), jnp.int32)
            dhb[tok, cs] = jnp.where(bits > 0, da, jnp.where(bits == 0, 0.5 * da, 0.0)).astype(BF)
        for g in range(G):
            r = slice(g * 128, (g + 1) * 128)
            ph, o, inv = phis[g], outs[g], invs[g]
            dnum3 = _heads(doT[r, :]) * inv
            dden = -jnp.sum(dnum3 * _heads(o), axis=1, keepdims=True)
            dden = _flat(jnp.broadcast_to(dden, dnum3.shape))
            dden = jnp.concatenate([dden, dden], axis=0)
            dnum = _flat(dnum3).astype(BF)
            dph = _nn(kvc[g], dnum) + dden * _lane_rep(zc[g])
            qT[0, r, tok] = _dual_softmax_bwd(ph[0:128], ph[128:256], dph[0:128], dph[128:256]).astype(BF)
            acc[g] += _nt(ph.astype(BF), dnum)
            zacc[g] += _lane_fold(ph * dden)
        return carry

    lax.fori_loop(0, NT, p2, 0)

    finish_state()
    wob[...] = dwo_acc[...].astype(BF)
    o_dwo = cp(wob, dwo_h, osem.at[2, 0])
    o_dwo.start()
    in_wv2 = cp(wqkv_h.at[:, 2 * D:3 * D], wT.at[2], isem.at[8])
    in_wv2.start()
    for j in range(2):
        for g in range(G):
            r = slice(g * 128, (g + 1) * 128)
            wT[j, :, r] = _nn(wqk[j, :, r], bd[r, :]).astype(BF)
    in_wv2.wait()

    def p3(t, carry):
        tok = pl.ds(pl.multiple_of(t * T, T), T)
        dxn = _nt(w1b[...], dhb[tok, :]) + _nn(wT[0], qT[0, :, tok])
        for g in range(G):
            r = slice(g * 128, (g + 1) * 128)
            phb = jnp.concatenate([qT[1, r, tok], qT[3, r, tok]], axis=0)
            dph = _nn(kvc[g], qT[2, r, tok]) + _lane_rep(zc[g])
            qT[2, r, tok] = _nn(kvT[g], phb).astype(BF)
            ph = phb.astype(F32)
            qT[1, r, tok] = _dual_softmax_bwd(ph[0:128], ph[128:256], dph[0:128], dph[128:256]).astype(BF)
        dxn = dxn + _nn(wT[2], qT[2, :, tok]) + _nn(wT[1], qT[1, :, tok])
        xn = xnT[:, tok].astype(F32)
        m1 = jnp.mean(dxn, axis=0, keepdims=True)
        m2 = jnp.mean(dxn * xn, axis=0, keepdims=True)
        dxT = (dxn - m1 - xn * m2) * rstdT[0:1, tok]
        gob[tok, :] = (gob[tok, :].astype(F32) + dxT.T).astype(BF)
        cp(gob.at[tok], dx_h.at[tok], osem.at[1, t]).start()
        return carry

    lax.fori_loop(0, NT, p3, 0)

    o_qkv = [cp(wT.at[j], dwqkv_h.at[:, j * D:(j + 1) * D], osem.at[2, 1 + j]) for j in range(3)]
    m = _head_mask(128)

    def p4a(g, carry):
        r = pl.ds(pl.multiple_of(g * 128, 128), 128)
        rhs = jnp.concatenate([qT[0, r, :], qT[1, r, :], qT[2, r, :]], axis=0)
        dw = _nt(xnT[...], rhs).astype(BF)
        dphi = jnp.zeros((128, 128), F32)
        for j in range(2):
            dwj = dw[:, j * 128:(j + 1) * 128]
            wT[j, :, r] = _nn(dwj, bdT[r, :]).astype(BF)
            dphi = dphi + _tn(wqk[j, :, r], dwj)
        wT[2, :, r] = dw[:, 256:384]
        dphi = jnp.where(m, dphi, 0.0)
        dphi = dphi[:, 0:32] + dphi[:, 32:64] + dphi[:, 64:96] + dphi[:, 96:128]
        dwphi_ref[r, :] = dphi.astype(BF)
        return carry

    lax.fori_loop(0, G, p4a, 0)
    for c in o_qkv:
        c.start()

    def p4b(c, carry):
        cs = pl.ds(pl.multiple_of(c * FC, FC), FC)
        w2b[cs, :] = _nn(dyT[...], ab[:, cs]).T.astype(BF)
        cp(w2b.at[cs, :], dw2_h.at[cs, :], osem.at[3, c]).start()
        w1b[:, cs] = _nn(xnT[...], dhb[:, cs]).astype(BF)
        cp(w1b.at[:, cs], dw1_h.at[:, cs], osem.at[4, c]).start()
        return carry

    lax.fori_loop(0, NF, p4b, 0)

    for t in range(NT):
        tok = pl.ds(t * T, T)
        cp(xb.at[tok], out_h.at[tok], osem.at[0, t]).wait()
        cp(gob.at[tok], dx_h.at[tok], osem.at[1, t]).wait()
    o_dwo.wait()
    for c in o_qkv:
        c.wait()
    for c in range(NF):
        cs = pl.ds(c * FC, FC)
        cp(w2b.at[cs, :], dw2_h.at[cs, :], osem.at[3, c]).wait()
        cp(w1b.at[:, cs], dw1_h.at[:, cs], osem.at[4, c]).wait()


@jax.jit
def pallas_recurrent_scan__linear_kernel_hedgehog__dense_activation_relu__prompt_kernel(
    A_x: jax.Array,
    A_wqkv: jax.Array,
    A_w_phi: jax.Array,
    A_wo: jax.Array,
    B_x: jax.Array,
    B_w1: jax.Array,
    B_w2: jax.Array,
    grad_out: jax.Array,
):
    del B_x
    hbm = pl.BlockSpec(memory_space=pl.ANY)
    vmem = pl.BlockSpec(memory_space=pltpu.VMEM)
    sds = jax.ShapeDtypeStruct
    out, dx, dwqkv, dwphi, dwo, dw1, dw2 = pl.pallas_call(
        _kernel,
        in_specs=[hbm, hbm, vmem, hbm, hbm, hbm, hbm],
        out_specs=[hbm, hbm, hbm, vmem, hbm, hbm, hbm],
        out_shape=[sds((S, D), BF), sds((S, D), BF), sds((D, 3 * D), BF), sds((D, DH), BF),
                   sds((D, D), BF), sds((D, F), BF), sds((F, D), BF)],
        scratch_shapes=[
            pltpu.VMEM((S, D), BF),
            pltpu.VMEM((S, D), BF),
            pltpu.VMEM((D, S), BF),
            pltpu.VMEM((S, F), BF),
            pltpu.VMEM((S, F), BF),
            pltpu.VMEM((D, S), BF),
            pltpu.VMEM((4, D, S), BF),
            pltpu.VMEM((D, F), BF),
            pltpu.VMEM((F, D), BF),
            pltpu.VMEM((3, D, D), BF),
            pltpu.VMEM((2, D, D), BF),
            pltpu.VMEM((D, D), BF),
            pltpu.VMEM((D, D), F32),
            pltpu.VMEM((D, 128), BF),
            pltpu.VMEM((D, 128), BF),
            pltpu.VMEM((8, S), F32),
            pltpu.VMEM((G, 256, 128), F32),
            pltpu.VMEM((G, 256, 128), F32),
            pltpu.VMEM((G, 128, 256), BF),
            pltpu.VMEM((G, 256, 128), BF),
            pltpu.VMEM((G, 256, 128), F32),
            pltpu.VMEM((G, 256, 128), F32),
            pltpu.SemaphoreType.DMA((9,)),
            pltpu.SemaphoreType.DMA((5, 8)),
        ],
        compiler_params=pltpu.CompilerParams(vmem_limit_bytes=127 * 1024 * 1024),
    )(A_x.reshape(S, D), A_wqkv, A_w_phi.reshape(D, DH), A_wo, B_w1, B_w2, grad_out.reshape(S, D))
    return (out.reshape(1, S, D), dx.reshape(1, S, D), dwqkv, dwphi.reshape(H, DH, DH), dwo, dw1, dw2)
```

```python
import jax
import jax.numpy as jnp
from jax import lax
import jax.experimental.pallas as pl
import jax.experimental.pallas.tpu as pltpu

S, D, H, DH, F = 2048, 1024, 32, 32, 3584
T = 256
NT = S // T
LB = 16
FC = 512
NF = F // FC
RING = S // FC
P = D // 64
G = D // 128
LOG2E = 1.4426950408889634
BF, F32 = jnp.bfloat16, jnp.float32


def _nn(a, b):
    return lax.dot_general(a, b, (((1,), (0,)), ((), ())), preferred_element_type=F32)


def _nt(a, b):
    return lax.dot_general(a, b, (((1,), (1,)), ((), ())), preferred_element_type=F32)


def _tn(a, b):
    return lax.dot_general(a, b, (((0,), (0,)), ((), ())), preferred_element_type=F32)


def _add(a, b):
    return (a.astype(F32) + b.astype(F32)).astype(BF)


def _sub(a, b):
    return (a.astype(F32) - b.astype(F32)).astype(BF)


def _sums(a, b, d, e):
    return [_add(a, e), _add(d, e), _add(a, b), _sub(d, a), _sub(b, e)]


def _put_sums(put, *blocks):
    rows, cols = blocks[0].shape
    w = min(cols, 256)
    h = 16 * 256 // w
    for r in range(0, rows, h):
        for c in range(0, cols, w):
            for i, v in enumerate(_sums(*[x[r:r + h, c:c + w] for x in blocks])):
                put(i, r, c, v)


def _sums_into(ref, *blocks, r0=0, c0=0):
    def put(i, r, c, v):
        ref[i, pl.ds(r0 + r, v.shape[0]), pl.ds(c0 + c, v.shape[1])] = v

    _put_sums(put, *blocks)
    return ref


def _strassen(dot, a11, a22, sa, b11, b22, sb, a_ready=True, between=lambda i: None):
    ops = {2: lambda: dot(sa[1], b11), 5: lambda: dot(sa[2], b22),
           4: lambda: dot(a22, sb[3]), 3: lambda: dot(a11, sb[4])}
    m = {}
    for i, k in enumerate((2, 5, 4, 3) if a_ready else (3, 4, 2, 5)):
        m[k] = ops[k]()
        between(i)
    c21 = m[2] + m[4]
    c12 = m[3] + m[5]
    m1 = dot(sa[0], sb[0])
    between(4)
    c11 = (m[4] - m[5] + m1) + dot(sa[4], sb[1])
    between(5)
    c22 = (m[3] - m[2] + m1) + dot(sa[3], sb[2])
    return c11, c12, c21, c22


def _join(c):
    return jnp.concatenate([jnp.concatenate(c[0:2], axis=1), jnp.concatenate(c[2:4], axis=1)], axis=0)


def _head_mask(rows, shift, m=3):
    r = lax.broadcasted_iota(jnp.int32, (rows, 128), 0)
    c = lax.broadcasted_iota(jnp.int32, (rows, 128), 1)
    return ((r >> shift) & m) == ((c >> shift) & m)


def _recip(x):
    r = pl.reciprocal(x, approx=True)
    return r * (2.0 - x * r)


def _gate(y, go):
    ey = jnp.exp(-jnp.abs(y))
    sig = _recip(1.0 + ey) * jnp.where(y >= 0.0, 1.0, ey)
    gate = y * sig
    go = go.astype(F32)
    return gate, go * gate, go * (sig + gate * (1.0 - sig))


def _by_rows(f, *xs):
    parts = [f(*[x[r:r + 16] for x in xs]) for r in range(0, xs[0].shape[0], 16)]
    return [jnp.concatenate(p, axis=0) for p in zip(*parts)]


def _heads(x):
    return x.reshape(x.shape[0] // DH, DH, x.shape[1])


def _flat(x):
    return x.reshape(x.shape[0] * DH, x.shape[2])


def _dual_softmax(p):
    p3 = _heads(p) * LOG2E
    ep = jnp.exp2(p3 - jnp.max(p3, axis=1, keepdims=True))
    em = jnp.exp2(jnp.min(p3, axis=1, keepdims=True) - p3)
    fp = ep * _recip(jnp.sum(ep, axis=1, keepdims=True))
    fm = em * _recip(jnp.sum(em, axis=1, keepdims=True))
    return jnp.concatenate([_flat(fp), _flat(fm)], axis=0)


def _dual_softmax_bwd(ph, dph):
    f, df = _heads(ph), _heads(dph)
    d = _flat(f * (df - jnp.sum(f * df, axis=1, keepdims=True)))
    n = d.shape[0] // 2
    return d[0:n] - d[n:2 * n]


def _lane_fold(x):
    acc = x[:, 0:128]
    for j in range(1, x.shape[1] // 128):
        acc = acc + x[:, j * 128:(j + 1) * 128]
    return acc


def _lane_rep(x):
    return jnp.concatenate([x] * (T // 128), axis=1)


def _center(x):
    x3 = _heads(x)
    return _flat(x3 - jnp.mean(x3, axis=1, keepdims=True))


def _kernel(x_h, wqkv_h, wphi_h, wo_h, w1_h, w2_h, go_h,
            out_h, dx_h, dwqkv_h, dwphi_h, dwo_h, dw1_h, dw2_h,
            xb, gob, xnb, xnT, ab, qT, w1b, w2b, wf, wob, xcur, swf, sa, sn,
            wpb, bd, bdT, rstdT, acc, zacc, kvT, kvc, zb, zc, isem, xsem, wsem, osem):
    def cp(src, dst, sem):
        return pltpu.make_async_copy(src, dst, sem)

    def tile(t):
        return pl.ds(t * T, T) if isinstance(t, int) else pl.ds(pl.multiple_of(t * T, T), T)

    def chunk(c):
        return pl.ds(c * FC, FC) if isinstance(c, int) else pl.ds(pl.multiple_of(c * FC, FC), FC)

    def halves(c):
        return [pl.ds(pl.multiple_of(c * FC + n * (FC // 2), FC // 2), FC // 2) for n in range(2)]

    HD, HS, HF, HT = D // 2, S // 2, F // 2, T // 2
    top, bot = slice(0, HD), slice(HD, D)
    f0, f1 = slice(0, HF), slice(HF, F)

    def half(t):
        return pl.ds(t * HT, HT) if isinstance(t, int) else pl.ds(pl.multiple_of(t * HT, HT), HT)

    def tile_halves(t):
        return half(2 * t), half(2 * t + 1)

    def wcat(r, k):
        return jnp.concatenate([wf[0, r, k], wf[1, r, k], wf[2, r, k]], axis=1)

    def strips(c):
        return [pl.ds(pl.multiple_of(c * (FC // 2) + n * HF, FC // 2), FC // 2) for n in range(2)]

    in_x = [cp(x_h.at[tile(t)], xb.at[tile(t)], xsem.at[t]) for t in range(NT)]
    quarter = [slice(i * 256, (i + 1) * 256) for i in range(4)]
    in_wk = cp(wqkv_h.at[:, D:2 * D], qT.at[0, :, D:2 * D], isem.at[1])
    in_wv = [cp(wqkv_h.at[:, pl.ds(2 * D + q.start, 256)], wf.at[2, :, q], wsem.at[i])
             for i, q in enumerate(quarter)]
    in_phi = cp(wphi_h, wpb, isem.at[0])
    o_phi = cp(wpb, dwphi_h, osem.at[0, 1])
    in_wq = cp(wqkv_h.at[:, 0:D], qT.at[0, :, 0:D], isem.at[3])
    in_w1a = cp(w1_h.at[:, 0:D], w1b.at[:, 0:D], isem.at[2])
    in_w1 = cp(w1_h.at[:, D:F], w1b.at[:, D:F], isem.at[4])
    in_w2 = cp(w2_h, w2b, isem.at[5])
    in_wo = cp(wo_h, wob, isem.at[6])
    in_go = cp(go_h, gob, isem.at[7])
    o_out = cp(xb, out_h, osem.at[0, 0])
    o_dwo = cp(wob, dwo_h, osem.at[2, 0])
    o_qkv = [cp(wf.at[j], dwqkv_h.at[:, j * D:(j + 1) * D], osem.at[2, 1 + j]) for j in range(3)]
    o_dx = cp(gob, dx_h, osem.at[1, 0])
    in_x[0].start()
    in_wv[0].start()
    in_wv[1].start()
    in_phi.start()
    acc[...] = jnp.zeros(acc.shape, F32)
    zacc[...] = jnp.zeros(zacc.shape, F32)

    def block_diag():
        for g in range(G):
            r = slice(g * 128, (g + 1) * 128)
            wbd = jnp.where(_head_mask(128, 5), jnp.concatenate([wpb[r, :].astype(F32)] * 4, axis=1), 0.0)
            bd[r, :] = wbd.astype(BF)
            bdT[r, :] = wbd.T.astype(BF)

    def fold(j):
        for g in range(G // 2):
            ra, rb = slice(g * 128, (g + 1) * 128), slice(HD + g * 128, HD + (g + 1) * 128)
            wa, wb = [_nn(qT[0, :, pl.ds(j * D + r.start, 128)], bd[r, :]) for r in (ra, rb)]
            wf[j, top, ra] = wa[top].astype(BF)
            wf[j, bot, rb] = wb[bot].astype(BF)
            _sums_into(swf.at[j], wa[top], wb[top], wa[bot], wb[bot], c0=g * 128)

    def layernorm(t):
        rs = [[], []]
        for i in range(0, HT, LB):
            xs = []
            for u in range(2):
                rows = pl.ds(tile(t).start + u * HT + i, LB)
                x = xb[rows, :].astype(F32)
                xc = x - jnp.mean(x, axis=1, keepdims=True)
                rstd = lax.rsqrt(jnp.mean(xc * xc, axis=1, keepdims=True) + 1e-5)
                xn = xc * rstd
                xnb[rows, :] = xn.astype(BF)
                xs += [xn[:, top], xn[:, bot]]
                rs[u].append(jnp.broadcast_to(rstd, (LB, 128)))
            _sums_into(sn, *xs, r0=half(t).start + i)
        rstdT[:, tile(t)] = jnp.concatenate(rs[0] + rs[1], axis=0).T[0:8, :]

    def xn_blocks(t):
        u0, u1 = tile_halves(t)
        return [sn[i, half(t), :] for i in range(5)] + [xnb[u0, top], xnb[u1, bot]]

    def project(x, j):
        c = _strassen(_nn, x[5], x[6], x, wf[j, top, top], wf[j, bot, bot], swf.at[j], False)
        return _join([c[0].T, c[2].T, c[1].T, c[3].T])

    def relu(h):
        return jnp.where(h < 0.0, -0.0, jnp.abs(h)).astype(BF)

    def v_first(i):
        qT[2, quarter[i], tile(0)] = _nn(xnb[tile(0), :], wf[2, :, quarter[i]]).T.astype(BF)

    in_x[0].wait()
    in_wv[2].start()
    layernorm(0)
    in_wv[0].wait()
    in_wv[3].start()
    in_phi.wait()
    v_first(0)
    block_diag()
    in_wv[1].wait()
    in_x[1].start()
    v_first(1)
    in_wv[2].wait()
    in_x[2].start()
    in_wv[3].wait()
    in_x[3].start()
    in_x[1].wait()
    in_wk.start()
    v_first(2)
    v_first(3)
    _sums_into(swf.at[2], wf[2, top, top], wf[2, top, bot], wf[2, bot, top], wf[2, bot, bot])

    def stage(t):
        layernorm(t)
        for i, v in enumerate(xn_blocks(t)):
            xcur[i] = v

    def p0(t, carry):
        cp(x_h.at[tile(t + 1)], xb.at[tile(t + 1)], xsem.at[t + 1]).wait()
        for when, later in ((1, in_x[4:6]), (2, in_x[6:8]), (3, [in_w1a]), (4, [in_wq]), (6, [in_w1])):
            @pl.when(t == when)
            def _():
                for c in later:
                    c.start()

        qT[2, :, tile(t)] = project(xcur, 2).astype(BF)
        stage(t + 1)
        return carry

    stage(1)
    lax.fori_loop(1, NT - 1, p0, 0)
    in_wk.wait()
    qT[2, :, tile(NT - 1)] = project(xcur, 2).astype(BF)
    fold(1)
    in_w1a.wait()
    in_w2.start()
    in_wo.start()

    def p1(t, carry):
        tok = tile(t)
        v = qT[2, :, tok]
        pk = project(xn_blocks(t), 1)
        xn = xnb[tok, :]
        xnT[:, tok] = xn.T
        for q, pairs in zip(quarter, (range(0, 5), range(5, 10), range(10, 16), ())):
            ab[t, :, :, q] = relu(_nn(xn, w1b[:, q])).reshape(2, HT, 256)
            for p in pairs:
                r = slice(p * 64, (p + 1) * 64)
                ph = _dual_softmax(pk[r, :])
                phb = ph.astype(BF)
                qT[1, r, tok] = phb[0:64]
                qT[3, r, tok] = phb[64:128]
                zacc[p] += _lane_fold(ph)
                acc[p] += _nt(v[r, :], phb)
        return carry

    lax.fori_loop(0, NT, p1, 0)

    def finish_state():
        m = _head_mask(64, 5, 1)
        for g in range(G):
            k0 = jnp.where(m, acc[2 * g], 0.0)
            k1 = jnp.where(m, acc[2 * g + 1], 0.0)
            kvT[2 * g] = k0.astype(BF)
            kvT[2 * g + 1] = k1.astype(BF)
            zero = jnp.zeros((64, 128), F32)
            kvc[g, 0:128] = _center(jnp.concatenate([k0, zero], axis=0).T).astype(BF)
            kvc[g, 128:256] = _center(jnp.concatenate([zero, k1], axis=0).T).astype(BF)
        for p in range(P):
            z = jnp.broadcast_to(jnp.sum(zacc[p], axis=1, keepdims=True), (128, 128))
            zb[p] = z
            zc[p] = _center(z)

    def forward_part(sw2, dwo_acc):
        def wo_sum(i, r=0, c=0, shape=(HD, HD)):
            return i // 2, pl.ds((i % 2) * HD + r, shape[0]), pl.ds((1 - i % 2) * HD + c, shape[1])

        def put_wo_sum(i, r, c, v):
            wf[wo_sum(i, r, c, v.shape)] = v

        def hidden(c):
            ab[:, :, :, chunk(c)] = relu(_nn(xnb[...], w1b[:, chunk(c)])).reshape(NT, 2, HT, FC)

        def p1b(c, carry):
            k0, k1 = [pl.ds(pl.multiple_of((c - 3) * (HF // 4) + n * HF, 64), HF // 4) for n in range(2)]
            _sums_into(sw2, w2b[k0, top], w2b[k0, bot], w2b[k1, top], w2b[k1, bot], r0=k0.start)
            hidden(c)
            return carry

        in_w1.wait()
        in_wq.wait()
        in_w2.wait()
        in_wo.wait()
        in_go.start()
        fold(0)
        hidden(2)
        _put_sums(put_wo_sum, wob[top, top], wob[top, bot], wob[bot, top], wob[bot, bot])
        finish_state()
        acc[...] = jnp.zeros(acc.shape, F32)
        zacc[...] = jnp.zeros(zacc.shape, F32)
        dwo_acc[...] = jnp.zeros(dwo_acc.shape, F32)
        lax.fori_loop(3, NF, p1b, 0)
        in_go.wait()

        def p2(t, carry):
            tok = tile(t)
            pq = project(xn_blocks(t), 0)
            phis, outs, invs = [], [], []

            def q_features(i):
                for p in range(*((0, 0), (0, 3), (3, 6), (6, 10), (10, 13), (13, 16))[i]):
                    ph = _dual_softmax(pq[p * 64:(p + 1) * 64, :])
                    pz = ph * _lane_rep(zb[p])
                    den = jnp.sum(_heads(pz[0:64] + pz[64:128]), axis=1, keepdims=True) + 1e-6
                    inv = _recip(den)
                    phis.append(ph)
                    outs.append(_flat(_heads(_nn(kvT[p], ph.astype(BF))) * inv))
                    invs.append(inv)

            acts = [ab[t, 0, :, f0], ab[t, 0, :, f1], ab[t, 1, :, f0], ab[t, 1, :, f1]]
            ys = _strassen(_nn, acts[0], acts[3], _sums(*acts), w2b[f0, top], w2b[f1, bot], sw2, False, q_features)
            oT = jnp.concatenate(outs, axis=0)
            o11, o12, o21, o22 = oT[top, 0:HT], oT[top, HT:T], oT[bot, 0:HT], oT[bot, HT:T]
            quad = [(pl.ds(pl.multiple_of(t * T + u * HT, HT), HT), k) for u in range(2) for k in (top, bot)]
            gates = [None] * 4
            for i in (2, 1, 0, 3):
                gates[i] = _by_rows(_gate, ys[i], gob[quad[i]])
            swo = [wf[wo_sum(i)] for i in range(5)]
            on = [v.T for v in (o11, o21, o12, o22)]
            ss = _strassen(_nn, on[0].astype(BF), on[3].astype(BF), _sums(*on),
                           wob[top, top], wob[bot, bot], swo, False)
            e11, e12, e21, e22 = [g[1] for g in gates]
            doT = _join(_strassen(_nt, wob[top, top], wob[bot, bot], swo,
                                  e11.astype(BF), e22.astype(BF), _sums(e11, e21, e12, e22)))
            for i in (2, 1, 0, 3):
                xb[quad[i]] = (xb[quad[i]].astype(F32) + ss[i] * gates[i][0]).astype(BF)
            d11, d12, d21, d22 = [ss[i] * gates[i][2] for i in range(4)]
            for i, d in enumerate(_sums(d11, d12, d21, d22) + [d11.astype(BF), d22.astype(BF)]):
                sn[i, half(t), :] = d
                sa[i, :, half(t)] = d.T

            def q_backward(step, _=None):
              for g in range(2 * step - 2, min(2 * step, G)) if step else ():
                dnums, ddens = [], []
                for p in (2 * g, 2 * g + 1):
                    dnum3 = _heads(doT[p * 64:(p + 1) * 64, :]) * invs[p]
                    dden = -jnp.sum(dnum3 * _heads(outs[p]), axis=1, keepdims=True)
                    dden = _flat(jnp.broadcast_to(dden, dnum3.shape))
                    ddens.append(jnp.concatenate([dden, dden], axis=0))
                    dnums.append(_flat(dnum3).astype(BF))
                dph2 = _nn(kvc[g], jnp.concatenate(dnums, axis=0))
                for i, p in enumerate((2 * g, 2 * g + 1)):
                    dph = dph2[i * 128:(i + 1) * 128] + ddens[i] * _lane_rep(zc[p])
                    qT[0, p * 64:(p + 1) * 64, tok] = _dual_softmax_bwd(phis[p], dph).astype(BF)
                    acc[p] += _nt(dnums[i], phis[p].astype(BF))
                    zacc[p] += _lane_fold(phis[p] * ddens[i])

            dws = _strassen(_nn, o11.astype(BF), o22.astype(BF), _sums(o11, o12, o21, o22),
                            e11.astype(BF), e22.astype(BF), _sums(e11, e12, e21, e22), True, q_backward)
            for b, v in zip([(top, top), (top, bot), (bot, top), (bot, bot)], dws):
                dwo_acc[b] += v
            return carry

        lax.fori_loop(0, NT, p2, 0)
        wob[...] = dwo_acc[...].astype(BF)

    pl.run_scoped(forward_part, pltpu.VMEM((5, HF, HD), BF), pltpu.VMEM((D, D), F32))

    def backward_part(sw1, dxn_b):
        def act_blocks(c):
            return [(slice(None), u, slice(None), n) for u in range(2) for n in halves(c)]

        def o_dw2(c):
            return cp(xnb.at[chunk(c % RING), :], dw2_h.at[chunk(c), :], osem.at[3, c])

        def p2w(c, carry):
            @pl.when(c >= RING)
            def _():
                o_dw2(c - RING).wait()

            acts = [ab[b].reshape(HS, FC // 2) for b in act_blocks(c)]
            dws = _strassen(lambda a, b: _nn(b, a), acts[0], acts[3],
                            _sums(acts[0], acts[2], acts[1], acts[3]), sa[5], sa[6], sa, False)
            n0, n1 = halves(c % RING)
            for b, dw in zip([(n0, top), (n0, bot), (n1, top), (n1, bot)], dws):
                xnb[b] = dw.T.astype(BF)
            o_dw2(c).start()
            return carry

        def p2b(c, carry):
            n0, n1 = halves(c)
            w11, w12, w21, w22 = w2b[n0, top], w2b[n1, top], w2b[n0, bot], w2b[n1, bot]
            das = _strassen(_nt, sn[5], sn[6], sn, w11, w22, _sums(w11, w12, w21, w22))
            for i in (2, 1, 0, 3):
                b = act_blocks(c)[i]
                bits = lax.bitcast_convert_type(ab[b].reshape(HS, FC // 2).astype(F32), jnp.int32)
                dh = jnp.where(bits > 0, das[i], jnp.where(bits == 0, 0.5 * das[i], 0.0))
                ab[b] = dh.astype(BF).reshape(NT, HT, FC // 2)
            k0, k1 = strips(c)
            _sums_into(sw1, w1b[top, k0], w1b[top, k1], w1b[bot, k0], w1b[bot, k1], c0=k0.start)
            return carry

        o_out.start()
        o_dwo.start()
        lax.fori_loop(0, NF, p2w, 0)
        finish_state()
        p2b(0, 0)
        o_out.wait()
        for c in range(NF - RING, NF):
            o_dw2(c).wait()
        lax.fori_loop(1, NF, p2b, 0)

        def p3(t, carry):
            tok = tile(t)
            u0, u1 = [pl.ds(pl.multiple_of(t * T + n * HT, HT), HT) for n in range(2)]
            x11, x22 = xnT[top, u0], xnT[bot, u1]
            _sums_into(sa, x11, xnT[top, u1], xnT[bot, u0], x22, c0=half(t).start)
            sa[5, :, half(t)] = x11
            sa[6, :, half(t)] = x22

            def kv_backward(step):
                for g in range(2 * step + 2, min(2 * step + 4, G)):
                    dph2 = _nn(kvc[g], qT[2, g * 128:(g + 1) * 128, tok])
                    for i, p in enumerate((2 * g, 2 * g + 1)):
                        r = slice(p * 64, (p + 1) * 64)
                        phb = jnp.concatenate([qT[1, r, tok], qT[3, r, tok]], axis=0)
                        dph = dph2[i * 128:(i + 1) * 128] + _lane_rep(zc[p])
                        qT[2, r, tok] = _nn(kvT[p], phb).astype(BF)
                        qT[1, r, tok] = _dual_softmax_bwd(phb.astype(F32), dph).astype(BF)

            kv_backward(-1)
            dh = [ab[t, 0, :, f0], ab[t, 1, :, f0], ab[t, 0, :, f1], ab[t, 1, :, f1]]
            c_ffn = _strassen(_nt, w1b[top, f0], w1b[bot, f1], sw1, dh[0], dh[3], _sums(*dh), True, kv_backward)
            dq = [qT[0:3, k, u].reshape(3 * HD, HT) for k in (top, bot) for u in (u0, u1)]
            lhs = [jnp.concatenate([swf[j, i] for j in range(3)], axis=1) for i in range(5)]
            c_att = _strassen(_nn, wcat(top, top), wcat(bot, bot), lhs, dq[0], dq[3], _sums(*dq))
            for b, v, w in zip([(top, u0), (top, u1), (bot, u0), (bot, u1)], c_ffn, c_att):
                dxn_b[b] = (v + w).astype(BF)
            return carry

        again = [cp(wqkv_h.at[:, j * D:(j + 1) * D], w2b.at[j * D:(j + 1) * D], isem.at[8 + j]) for j in range(2)]
        for c in again:
            c.start()
        lax.fori_loop(0, NT, p3, 0)
        for c in again:
            c.wait()

        def layernorm_bwd(t):
            tok = tile(t)
            dxn = dxn_b[:, tok].astype(F32)
            xn = xnT[:, tok].astype(F32)
            m1 = jnp.mean(dxn, axis=0, keepdims=True)
            m2 = jnp.mean(dxn * xn, axis=0, keepdims=True)
            dxT = (dxn - m1 - xn * m2) * rstdT[0:1, tok]
            gob[tok, :] = (gob[tok, :].astype(F32) + dxT.T).astype(BF)

        def p4a(i, carry):
            layernorm_bwd(2 * i)
            layernorm_bwd(2 * i + 1)
            rs = [pl.ds(pl.multiple_of((2 * i + n) * 128, 128), 128) for n in range(2)]
            full = [jnp.concatenate([qT[0, r, :], qT[1, r, :], qT[2, r, :]], axis=0) for r in rs]
            b11, b12, b21, b22 = [
                jnp.concatenate([f[:, t * T + u * HT:t * T + (u + 1) * HT] for t in range(NT)], axis=1)
                for u in range(2) for f in full]
            c11, c12, c21, c22 = _strassen(_nt, sa[5], sa[6], sa, b11, b22,
                                           _sums(b11, b12, b21, b22))
            for rows, r, dw in ((bot, rs[0], c21), (top, rs[1], c12), (top, rs[0], c11), (bot, rs[1], c22)):
                for j in range(3):
                    wf[j, rows, r] = dw[:, j * 128:(j + 1) * 128].astype(BF)
            return carry

        def unfold(g):
            r = pl.ds(pl.multiple_of(g * 128, 128), 128)
            dphi = jnp.zeros((128, 128), F32)
            for j in range(2):
                dwj = wf[j, :, r]
                dphi = dphi + _tn(w2b[j * D:(j + 1) * D, r], dwj)
                wf[j, :, r] = _nn(dwj, bdT[r, :]).astype(BF)
            dphi = jnp.where(_head_mask(128, 5), dphi, 0.0)
            dphi = dphi[:, 0:32] + dphi[:, 32:64] + dphi[:, 64:96] + dphi[:, 96:128]
            wpb[r, :] = dphi.astype(BF)

        def p4b(c, carry, between=lambda i: None):
            n0, n1 = halves(c)
            b11, b12, b21, b22 = [ab[:, u, :, n].reshape(HS, FC // 2) for u in range(2) for n in (n0, n1)]
            c11, c12, c21, c22 = _strassen(_nn, sa[5], sa[6], sa, b11, b22,
                                           _sums(b11, b12, b21, b22), True, between)
            for i, (rows, n, v) in enumerate(((bot, n0, c21), (top, n1, c12), (top, n0, c11), (bot, n1, c22))):
                w1b[rows, n] = v.astype(BF)
                cp(w1b.at[rows, n], dw1_h.at[rows, n], osem.at[4 + i, c]).start()
            return carry

        lax.fori_loop(0, G // 2, p4a, 0)
        o_dx.start()
        o_qkv[2].start()

        def p4u(c, carry):
            return p4b(c, carry, lambda i: unfold(2 * c + i) if i < 2 else None)

        lax.fori_loop(0, G // 2, p4u, 0)
        o_qkv[0].start()
        o_qkv[1].start()
        o_phi.start()
        lax.fori_loop(G // 2, NF, p4b, 0)

    pl.run_scoped(backward_part, pltpu.VMEM((5, HD, HF), BF), pltpu.VMEM((D, S), BF))

    o_dx.wait()
    o_dwo.wait()
    o_phi.wait()
    for c in o_qkv:
        c.wait()
    for c in range(NF):
        n0, n1 = halves(c)
        for i, (rows, n) in enumerate(((bot, n0), (top, n1), (top, n0), (bot, n1))):
            cp(w1b.at[rows, n], dw1_h.at[rows, n], osem.at[4 + i, c]).wait()


@jax.jit
def pallas_recurrent_scan__linear_kernel_hedgehog__dense_activation_relu__prompt_kernel(
    A_x: jax.Array,
    A_wqkv: jax.Array,
    A_w_phi: jax.Array,
    A_wo: jax.Array,
    B_x: jax.Array,
    B_w1: jax.Array,
    B_w2: jax.Array,
    grad_out: jax.Array,
):
    del B_x
    hbm = pl.BlockSpec(memory_space=pl.ANY)
    sds = jax.ShapeDtypeStruct
    out, dx, dwqkv, dwphi, dwo, dw1, dw2 = pl.pallas_call(
        _kernel,
        in_specs=[hbm] * 7,
        out_specs=[hbm] * 7,
        out_shape=[sds((S, D), BF), sds((S, D), BF), sds((D, 3 * D), BF), sds((D, DH), BF),
                   sds((D, D), BF), sds((D, F), BF), sds((F, D), BF)],
        scratch_shapes=[
            pltpu.VMEM((S, D), BF),
            pltpu.VMEM((S, D), BF),
            pltpu.VMEM((S, D), BF),
            pltpu.VMEM((D, S), BF),
            pltpu.VMEM((NT, 2, T // 2, F), BF),
            pltpu.VMEM((4, D, S), BF),
            pltpu.VMEM((D, F), BF),
            pltpu.VMEM((F, D), BF),
            pltpu.VMEM((3, D, D), BF),
            pltpu.VMEM((D, D), BF),
            pltpu.VMEM((7, T // 2, D // 2), BF),
            pltpu.VMEM((3, 5, D // 2, D // 2), BF),
            pltpu.VMEM((7, D // 2, S // 2), BF),
            pltpu.VMEM((7, S // 2, D // 2), BF),
            pltpu.VMEM((D, DH), BF),
            pltpu.VMEM((D, 128), BF),
            pltpu.VMEM((D, 128), BF),
            pltpu.VMEM((8, S), F32),
            pltpu.VMEM((P, 64, 128), F32),
            pltpu.VMEM((P, 128, 128), F32),
            pltpu.VMEM((P, 64, 128), BF),
            pltpu.VMEM((G, 256, 128), BF),
            pltpu.VMEM((P, 128, 128), F32),
            pltpu.VMEM((P, 128, 128), F32),
            pltpu.SemaphoreType.DMA((10,)),
            pltpu.SemaphoreType.DMA((NT,)),
            pltpu.SemaphoreType.DMA((4,)),
            pltpu.SemaphoreType.DMA((8, 8)),
        ],
        compiler_params=pltpu.CompilerParams(vmem_limit_bytes=127 * 1024 * 1024,
                                             flags={"XLA_TPU_EVENLY_DISTRIBUTE_CRITICAL_NODES": True}),
    )(A_x.reshape(S, D), A_wqkv, A_w_phi.reshape(D, DH), A_wo, B_w1, B_w2, grad_out.reshape(S, D))
    return (out.reshape(1, S, D), dx.reshape(1, S, D), dwqkv, dwphi.reshape(H, DH, DH), dwo, dw1, dw2)
```

```python
import jax
import jax.numpy as jnp
from jax import lax
import jax.experimental.pallas as pl
import jax.experimental.pallas.tpu as pltpu

S, D, H, DH, F = 2048, 1024, 32, 32, 3584
T = 256
NT = S // T
LB = 16
FC = 512
NF = F // FC
RING = S // FC
P = D // 64
G = D // 128
LOG2E = 1.4426950408889634
BF, F32 = jnp.bfloat16, jnp.float32


def _nn(a, b):
    return lax.dot_general(a, b, (((1,), (0,)), ((), ())), preferred_element_type=F32)


def _nt(a, b):
    return lax.dot_general(a, b, (((1,), (1,)), ((), ())), preferred_element_type=F32)


def _tn(a, b):
    return lax.dot_general(a, b, (((0,), (0,)), ((), ())), preferred_element_type=F32)


def _add(a, b):
    return (a.astype(F32) + b.astype(F32)).astype(BF)


def _sub(a, b):
    return (a.astype(F32) - b.astype(F32)).astype(BF)


def _sums(a, b, d, e):
    return [_add(a, e), _add(d, e), _add(a, b), _sub(d, a), _sub(b, e)]


def _put_sums(put, *blocks):
    rows, cols = blocks[0].shape
    w = min(cols, 256)
    h = 16 * 256 // w
    for r in range(0, rows, h):
        for c in range(0, cols, w):
            for i, v in enumerate(_sums(*[x[r:r + h, c:c + w] for x in blocks])):
                put(i, r, c, v)


def _sums_into(ref, *blocks, r0=0, c0=0):
    def put(i, r, c, v):
        ref[i, pl.ds(r0 + r, v.shape[0]), pl.ds(c0 + c, v.shape[1])] = v

    _put_sums(put, *blocks)
    return ref


def _strassen(dot, a11, a22, sa, b11, b22, sb, a_ready=True, between=lambda i, *c: None, done=None):
    ops = {2: lambda: dot(sa[1], b11), 5: lambda: dot(sa[2], b22),
           4: lambda: dot(a22, sb[3]), 3: lambda: dot(a11, sb[4])}
    m = dict(done or {})
    for i, k in enumerate((2, 5, 4, 3) if a_ready else (3, 4, 2, 5)):
        if k not in m:
            m[k] = ops[k]()
        between(i)
    c21 = m[2] + m[4]
    c12 = m[3] + m[5]
    m1 = m[1] if 1 in m else dot(sa[0], sb[0])
    between(4, c21)
    c11 = (m[4] - m[5] + m1) + dot(sa[4], sb[1])
    between(5, c12)
    c22 = (m[3] - m[2] + m1) + dot(sa[3], sb[2])
    return c11, c12, c21, c22


def _join(c):
    return jnp.concatenate([jnp.concatenate(c[0:2], axis=1), jnp.concatenate(c[2:4], axis=1)], axis=0)


def _head_mask(rows, shift, m=3):
    r = lax.broadcasted_iota(jnp.int32, (rows, 128), 0)
    c = lax.broadcasted_iota(jnp.int32, (rows, 128), 1)
    return ((r >> shift) & m) == ((c >> shift) & m)


def _recip(x):
    r = pl.reciprocal(x, approx=True)
    return r * (2.0 - x * r)


def _gate(y, go):
    ey = jnp.exp(-jnp.abs(y))
    sig = _recip(1.0 + ey) * jnp.where(y >= 0.0, 1.0, ey)
    gate = y * sig
    go = go.astype(F32)
    return gate, go * gate, go * (sig + gate * (1.0 - sig))


def _by_rows(f, *xs):
    parts = [f(*[x[r:r + 16] for x in xs]) for r in range(0, xs[0].shape[0], 16)]
    return [jnp.concatenate(p, axis=0) for p in zip(*parts)]


def _heads(x):
    return x.reshape(x.shape[0] // DH, DH, x.shape[1])


def _flat(x):
    return x.reshape(x.shape[0] * DH, x.shape[2])


def _dual_softmax(p):
    p3 = _heads(p) * LOG2E
    ep = jnp.exp2(p3 - jnp.max(p3, axis=1, keepdims=True))
    em = jnp.exp2(jnp.min(p3, axis=1, keepdims=True) - p3)
    fp = ep * _recip(jnp.sum(ep, axis=1, keepdims=True))
    fm = em * _recip(jnp.sum(em, axis=1, keepdims=True))
    return jnp.concatenate([_flat(fp), _flat(fm)], axis=0)


def _dual_softmax_bwd(ph, dph):
    f, df = _heads(ph), _heads(dph)
    d = _flat(f * (df - jnp.sum(f * df, axis=1, keepdims=True)))
    n = d.shape[0] // 2
    return d[0:n] - d[n:2 * n]


def _lane_fold(x):
    acc = x[:, 0:128]
    for j in range(1, x.shape[1] // 128):
        acc = acc + x[:, j * 128:(j + 1) * 128]
    return acc


def _lane_rep(x):
    return jnp.concatenate([x] * (T // 128), axis=1)


def _center(x):
    x3 = _heads(x)
    return _flat(x3 - jnp.mean(x3, axis=1, keepdims=True))


def _kernel(x_h, wqkv_h, wphi_h, wo_h, w1_h, w2_h, go_h,
            out_h, dx_h, dwqkv_h, dwphi_h, dwo_h, dw1_h, dw2_h,
            xb, gob, xnb, ab, qT, w1b, w2b, wf, wob, swf, sa, sn,
            wpb, bd, rstdT, acc, zacc, kvT, zb, isem, xsem, wsem, osem):
    def cp(src, dst, sem):
        return pltpu.make_async_copy(src, dst, sem)

    def tile(t):
        return pl.ds(t * T, T) if isinstance(t, int) else pl.ds(pl.multiple_of(t * T, T), T)

    def chunk(c):
        return pl.ds(c * FC, FC) if isinstance(c, int) else pl.ds(pl.multiple_of(c * FC, FC), FC)

    def halves(c):
        return [pl.ds(pl.multiple_of(c * FC + n * (FC // 2), FC // 2), FC // 2) for n in range(2)]

    HD, HS, HF, HT = D // 2, S // 2, F // 2, T // 2
    top, bot = slice(0, HD), slice(HD, D)
    f0, f1 = slice(0, HF), slice(HF, F)

    def half(t):
        return pl.ds(t * HT, HT) if isinstance(t, int) else pl.ds(pl.multiple_of(t * HT, HT), HT)

    def tile_halves(t):
        return half(2 * t), half(2 * t + 1)

    def strips(c):
        return [pl.ds(pl.multiple_of(c * (FC // 2) + n * HF, FC // 2), FC // 2) for n in range(2)]

    in_x = [cp(x_h.at[tile(t)], xb.at[tile(t)], xsem.at[t]) for t in range(NT)]
    quarter = [slice(i * 256, (i + 1) * 256) for i in range(4)]
    in_wk = cp(wqkv_h.at[:, D:2 * D], qT.at[0, :, D:2 * D], isem.at[1])
    in_wv = [cp(wqkv_h.at[:, pl.ds(2 * D + q.start, 256)], wf.at[2, :, q], wsem.at[i])
             for i, q in enumerate(quarter)]
    in_phi = cp(wphi_h, wpb, isem.at[0])
    o_phi = cp(wpb, dwphi_h, osem.at[0, 1])
    in_wq = cp(wqkv_h.at[:, 0:D], qT.at[0, :, 0:D], isem.at[3])
    in_w1a = cp(w1_h.at[:, 0:D], w1b.at[:, 0:D], isem.at[2])
    in_w1 = cp(w1_h.at[:, D:F], w1b.at[:, D:F], isem.at[4])
    in_w2 = cp(w2_h, w2b, isem.at[5])
    in_wo = cp(wo_h, wob, isem.at[6])
    in_go = cp(go_h, gob, isem.at[7])
    o_out = cp(xb, out_h, osem.at[0, 0])
    o_dwo = cp(wob, dwo_h, osem.at[2, 0])
    o_qkv = [cp(wf.at[j], dwqkv_h.at[:, j * D:(j + 1) * D], osem.at[2, 1 + j]) for j in range(3)]
    o_dx = cp(gob, dx_h, osem.at[1, 0])
    in_phi.start()
    in_x[0].start()
    in_wv[0].start()
    acc[...] = jnp.zeros(acc.shape, F32)
    zacc[...] = jnp.zeros(zacc.shape, F32)

    def block_diag():
        for g in range(G):
            r = slice(g * 128, (g + 1) * 128)
            wbd = jnp.where(_head_mask(128, 5), jnp.concatenate([wpb[r, :].astype(F32)] * 4, axis=1), 0.0)
            bd[r, :] = wbd.astype(BF)

    def fold(j):
        for g in range(G // 2):
            ra, rb = slice(g * 128, (g + 1) * 128), slice(HD + g * 128, HD + (g + 1) * 128)
            wa, wb = [_nn(qT[0, :, pl.ds(j * D + r.start, 128)], bd[r, :]) for r in (ra, rb)]
            wf[j, top, ra] = wa[top].astype(BF)
            wf[j, bot, rb] = wb[bot].astype(BF)
            _sums_into(swf.at[j], wa[top], wb[top], wa[bot], wb[bot], c0=g * 128)

    def layernorm(t):
        rs = [[], []]
        for i in range(0, HT, LB):
            xs = []
            for u in range(2):
                rows = pl.ds(tile(t).start + u * HT + i, LB)
                x = xb[rows, :].astype(F32)
                xc = x - jnp.mean(x, axis=1, keepdims=True)
                rstd = lax.rsqrt(jnp.mean(xc * xc, axis=1, keepdims=True) + 1e-5)
                xn = xc * rstd
                xnb[rows, :] = xn.astype(BF)
                xs += [xn[:, top], xn[:, bot]]
                rs[u].append(jnp.broadcast_to(rstd, (LB, 128)))
            sums = _sums(*xs)
            for n, v in enumerate(sums):
                sn[n, pl.ds(half(t).start + i, LB), :] = v
        rstdT[:, tile(t)] = jnp.concatenate(rs[0] + rs[1], axis=0).T[0:8, :]

    def xn_blocks(t):
        u0, u1 = tile_halves(t)
        return [sn[i, half(t), :] for i in range(5)] + [xnb[u0, top], xnb[u1, bot]]

    def project(x, j):
        c = _strassen(_nn, x[5], x[6], x, wf[j, top, top], wf[j, bot, bot], swf.at[j], False)
        return _join([c[0].T, c[2].T, c[1].T, c[3].T])

    def relu(h):
        return jnp.where(h < 0.0, -0.0, jnp.abs(h)).astype(BF)

    def v_first(i):
        qT[2, quarter[i], tile(0)] = _nn(xnb[tile(0), :], wf[2, :, quarter[i]]).T.astype(BF)

    in_phi.wait()
    in_wv[1].start()
    block_diag()
    in_x[0].wait()
    in_x[1].start()
    layernorm(0)
    in_wv[0].wait()
    in_wv[2].start()
    in_wv[3].start()
    v_first(0)
    in_wv[1].wait()
    in_x[1].wait()
    in_x[2].start()
    in_x[3].start()
    v_first(1)
    layernorm(1)
    in_wv[2].wait()
    in_wv[3].wait()
    in_x[4].start()
    in_x[5].start()
    v_first(2)
    v_first(3)
    _sums_into(swf.at[2], wf[2, top, top], wf[2, top, bot], wf[2, bot, top], wf[2, bot, bot])

    later = {1: in_x[6:8], 2: [in_wk], 4: [in_w1a, in_wq], 6: [in_w1]}
    for t in range(1, NT):
        for c in {1: in_x[2:3], 2: in_x[3:5], 4: in_x[5:7], 6: [in_x[7], in_wk]}.get(t, ()):
            c.wait()
        for c in later.get(t, ()):
            c.start()
        if t + 1 < NT:
            layernorm(t + 1)
        qT[2, :, tile(t)] = project(xn_blocks(t), 2).astype(BF)
    fold(1)
    in_w1a.wait()
    in_w2.start()
    in_wo.start()

    def p1(t, carry):
        tok = tile(t)
        v = qT[2, :, tok]
        pk = project(xn_blocks(t), 1)
        xn = xnb[tok, :]
        for q, pairs in zip(quarter, (range(0, 4), range(4, 8), range(8, 12), range(12, 16))):
            ab[t, :, :, q] = relu(_nn(xn, w1b[:, q])).reshape(2, HT, 256)
            for p in pairs:
                r = slice(p * 64, (p + 1) * 64)
                ph = _dual_softmax(pk[r, :])
                phb = ph.astype(BF)
                qT[1, r, tok] = phb[0:64]
                qT[3, r, tok] = phb[64:128]
                zacc[p] += _lane_fold(ph)
                acc[p] += _nt(v[r, :], phb)
        return carry

    lax.fori_loop(0, NT, p1, 0)

    def kv_slot(g):
        return 2, pl.ds(HD + (g // 4) * 256, 256), pl.ds((g % 4) * 128, 128)

    def finish_state(center_z):
        m = _head_mask(64, 5, 1)
        for g in range(G):
            k0 = jnp.where(m, acc[2 * g], 0.0)
            k1 = jnp.where(m, acc[2 * g + 1], 0.0)
            kvT[2 * g] = k0.astype(BF)
            kvT[2 * g + 1] = k1.astype(BF)
            zero = jnp.zeros((64, 128), F32)
            wf[kv_slot(g)] = _center(_join([k0, zero, zero, k1]).T).astype(BF)
        for p in range(P):
            z = jnp.broadcast_to(jnp.sum(zacc[p], axis=1, keepdims=True), (128, 128))
            zb[p] = _center(z) if center_z else z

    def forward_part(sw2, dwo_acc):
        def wo_sum(i, r=0, c=0, shape=(HD, HD)):
            return i // 2, pl.ds((i % 2) * HD + r, shape[0]), pl.ds((1 - i % 2) * HD + c, shape[1])

        def put_wo_sum(i, r, c, v):
            wf[wo_sum(i, r, c, v.shape)] = v

        def hidden(c):
            ab[:, :, :, chunk(c)] = relu(_nn(xnb[...], w1b[:, chunk(c)])).reshape(NT, 2, HT, FC)

        def p1b(c, carry):
            k0, k1 = [pl.ds(pl.multiple_of((c - 3) * (HF // 4) + n * HF, 64), HF // 4) for n in range(2)]
            _sums_into(sw2, w2b[k0, top], w2b[k0, bot], w2b[k1, top], w2b[k1, bot], r0=k0.start)
            hidden(c)
            return carry

        in_w1.wait()
        in_wq.wait()
        in_w2.wait()
        in_wo.wait()
        in_go.start()
        fold(0)
        hidden(2)
        _put_sums(put_wo_sum, wob[top, top], wob[top, bot], wob[bot, top], wob[bot, bot])
        finish_state(False)
        acc[...] = jnp.zeros(acc.shape, F32)
        zacc[...] = jnp.zeros(zacc.shape, F32)
        dwo_acc[...] = jnp.zeros(dwo_acc.shape, F32)
        lax.fori_loop(3, NF, p1b, 0)
        in_go.wait()

        def p2(t, carry):
            tok = tile(t)
            pq = project(xn_blocks(t), 0)
            phis, outs, invs = [], [], []

            quad = [(u, k) for u in tile_halves(t) for k in (top, bot)]
            swo = [wf[wo_sum(i)] for i in range(5)]
            gates, early = [None] * 4, {}

            def q_features(i, y=None):
                if i == 4:
                    gates[0] = _by_rows(_gate, y, gob[quad[0]])
                    early[2] = _nt(swo[1], gates[0][1].astype(BF))
                if i == 5:
                    gates[3] = _by_rows(_gate, y, gob[quad[3]])
                    early[5] = _nt(swo[2], gates[3][1].astype(BF))
                for p in range(*((0, 2), (2, 5), (5, 9), (9, 13), (13, 15), (15, 16))[i]):
                    ph = _dual_softmax(pq[p * 64:(p + 1) * 64, :])
                    pz = ph * _lane_rep(zb[p])
                    den = jnp.sum(_heads(pz[0:64] + pz[64:128]), axis=1, keepdims=True) + 1e-6
                    inv = _recip(den)
                    phis.append(ph)
                    outs.append(_flat(_heads(_nn(kvT[p], ph.astype(BF))) * inv))
                    invs.append(inv)

            acts = [ab[t, 1, :, f0], ab[t, 1, :, f1], ab[t, 0, :, f0], ab[t, 0, :, f1]]
            ys = _strassen(_nn, acts[0], acts[3], _sums(*acts), w2b[f0, top], w2b[f1, bot], sw2, False, q_features)
            oT = jnp.concatenate(outs, axis=0)
            o11, o12, o21, o22 = oT[top, 0:HT], oT[top, HT:T], oT[bot, 0:HT], oT[bot, HT:T]
            gates[2] = _by_rows(_gate, ys[0], gob[quad[2]])
            gates[1] = _by_rows(_gate, ys[3], gob[quad[1]])
            on = [v.T for v in (o11, o21, o12, o22)]
            ss = _strassen(_nn, on[0].astype(BF), on[3].astype(BF), _sums(*on),
                           wob[top, top], wob[bot, bot], swo, False)
            e11, e12, e21, e22 = [g[1] for g in gates]
            doT = _join(_strassen(_nt, wob[top, top], wob[bot, bot], swo,
                                  e11.astype(BF), e22.astype(BF), _sums(e11, e21, e12, e22), done=early))
            for i in (2, 1, 0, 3):
                xb[quad[i]] = (xb[quad[i]].astype(F32) + ss[i] * gates[i][0]).astype(BF)
            d11, d12, d21, d22 = [ss[i] * gates[i][2] for i in range(4)]
            for i, d in enumerate(_sums(d11, d12, d21, d22) + [d11.astype(BF), d22.astype(BF)]):
                sn[i, half(t), :] = d
                sa[i, :, half(t)] = d.T

            def q_backward(step, _=None):
                for g in range(*((0, 0), (0, 1), (1, 3), (3, 5), (5, 7), (7, 8))[step]):
                    dnums, ddens = [], []
                    for p in (2 * g, 2 * g + 1):
                        dnum3 = _heads(doT[p * 64:(p + 1) * 64, :]) * invs[p]
                        dden = -jnp.sum(dnum3 * _heads(outs[p]), axis=1, keepdims=True)
                        dden = _flat(jnp.broadcast_to(dden, dnum3.shape))
                        ddens.append(jnp.concatenate([dden, dden], axis=0))
                        dnums.append(_flat(dnum3).astype(BF))
                    dph2 = _nn(wf[kv_slot(g)], jnp.concatenate(dnums, axis=0))
                    for i, p in enumerate((2 * g, 2 * g + 1)):
                        dph = dph2[i * 128:(i + 1) * 128] + ddens[i] * _lane_rep(zb[p])
                        qT[0, p * 64:(p + 1) * 64, tok] = _dual_softmax_bwd(phis[p], dph).astype(BF)
                        acc[p] += _nt(dnums[i], phis[p].astype(BF))
                        zacc[p] += _lane_fold(phis[p] * ddens[i])

            dws = _strassen(_nn, o11.astype(BF), o22.astype(BF), _sums(o11, o12, o21, o22),
                            e11.astype(BF), e22.astype(BF), _sums(e11, e12, e21, e22), True, q_backward)
            for b, v in zip([(bot, top), (top, bot), (top, top), (bot, bot)], [dws[i] for i in (2, 1, 0, 3)]):
                dwo_acc[b] += v
            return carry

        lax.fori_loop(0, NT, p2, 0)
        wob[...] = dwo_acc[...].astype(BF)

    pl.run_scoped(forward_part, pltpu.VMEM((5, HF, HD), BF), pltpu.VMEM((D, D), F32))

    def backward_part(sw1, xnT):
        def act_blocks(c):
            return [(slice(None), u, slice(None), n) for u in range(2) for n in halves(c)]

        def o_dw2(c):
            return cp(xnT.at[(c // 2) % 2, chunk(c % 2), :], dw2_h.at[chunk(c), :], osem.at[3, c])

        def p2w(c, carry):
            @pl.when(c >= RING)
            def _():
                o_dw2(c - RING).wait()

            acts = [ab[b].reshape(HS, FC // 2) for b in act_blocks(c)]
            dws = _strassen(lambda a, b: _nn(b, a), acts[0], acts[3],
                            _sums(acts[0], acts[2], acts[1], acts[3]), sa[5], sa[6], sa, False)
            n0, n1 = halves(c % 2)
            for b, dw in (((n0, bot), dws[1]), ((n1, top), dws[2]), ((n0, top), dws[0]), ((n1, bot), dws[3])):
                xnT[((c // 2) % 2,) + b] = dw.T.astype(BF)
            o_dw2(c).start()
            return carry

        def p2b(c, carry):
            n0, n1 = halves(c)
            w11, w12, w21, w22 = w2b[n0, top], w2b[n1, top], w2b[n0, bot], w2b[n1, bot]
            das = _strassen(_nt, sn[5], sn[6], sn, w11, w22, _sums(w11, w12, w21, w22))
            for i in (2, 1, 0, 3):
                b = act_blocks(c)[i]
                bits = lax.bitcast_convert_type(ab[b].reshape(HS, FC // 2).astype(F32), jnp.int32)
                dh = jnp.where(bits > 0, das[i], jnp.where(bits == 0, 0.5 * das[i], 0.0))
                ab[b] = dh.astype(BF).reshape(NT, HT, FC // 2)
            k0, k1 = strips(c)
            for r in range(0, HD, 16):
                ra, rb = slice(r, r + 16), slice(HD + r, HD + r + 16)
                v = _sums(w1b[ra, k0], w1b[ra, k1], w1b[rb, k0], w1b[rb, k1])
                for i in range(3):
                    sw1[i, ra, k0] = v[i]
                w1b[rb, k0] = v[3]
                w1b[ra, k1] = v[4]
            return carry

        o_out.start()
        o_dwo.start()
        lax.fori_loop(0, NF, p2w, 0)
        finish_state(True)
        p2b(0, 0)
        o_out.wait()
        for c in range(NF - RING, NF):
            o_dw2(c).wait()
        lax.fori_loop(1, NF, p2b, 0)

        def p3(t, carry):
            tok = tile(t)
            u0, u1 = [pl.ds(pl.multiple_of(t * T + n * HT, HT), HT) for n in range(2)]
            xt = [xnb[u0, :].T, xnb[u1, :].T]
            xnT[0, :, half(t)] = xt[0]
            xnT[1, :, half(t)] = xt[1]
            x11, x22 = xt[0][top], xt[1][bot]
            _sums_into(sa, x11, xt[1][top], xt[0][bot], x22, c0=half(t).start)
            sa[5, :, half(t)] = x11
            sa[6, :, half(t)] = x22

            def kv_backward(step, _=None):
                for g in range(*((0, 1), (1, 2), (2, 4), (4, 5), (5, 6), (6, 7), (7, 8))[step + 1]):
                    dph2 = _nn(wf[kv_slot(g)], qT[2, g * 128:(g + 1) * 128, tok])
                    for i, p in enumerate((2 * g, 2 * g + 1)):
                        r = slice(p * 64, (p + 1) * 64)
                        phb = jnp.concatenate([qT[1, r, tok], qT[3, r, tok]], axis=0)
                        dph = dph2[i * 128:(i + 1) * 128] + _lane_rep(zb[p])
                        qT[2, r, tok] = _nn(kvT[p], phb).astype(BF)
                        qT[1, r, tok] = _dual_softmax_bwd(phb.astype(F32), dph).astype(BF)

            kv_backward(-1)
            dh = [ab[t, 0, :, f0], ab[t, 1, :, f0], ab[t, 0, :, f1], ab[t, 1, :, f1]]
            c_ffn = _strassen(_nt, w1b[top, f0], w1b[bot, f1], [sw1[0], sw1[1], sw1[2], w1b[bot, f0], w1b[top, f1]],
                              dh[0], dh[3], _sums(*dh), True, kv_backward)
            for j in (0, 2, 1):
                dq = [qT[j, k, u] for k in (top, bot) for u in (u0, u1)]
                c_att = _strassen(_nn, wf[j, top, top], wf[j, bot, bot], swf.at[j], dq[0], dq[3], _sums(*dq))
                c_ffn = [v + w for v, w in zip(c_ffn, c_att)]
            v0, v1 = tile_halves(t % 2)
            for b, v in zip([(bot, v0), (top, v1), (top, v0), (bot, v1)], [c_ffn[i] for i in (2, 1, 0, 3)]):
                sn[(t // 2,) + b] = v.astype(BF)
            return carry

        again = [cp(wqkv_h.at[:, j * D:(j + 1) * D], w2b.at[j * D:(j + 1) * D], isem.at[8 + j]) for j in range(2)]
        for c in again:
            c.start()
        lax.fori_loop(0, NT, p3, 0)
        for c in again:
            c.wait()

        def layernorm_bwd(i, n):
            t = 2 * i + n
            tok = tile(t)
            dxn = sn[i, :, tile(n)].astype(F32)
            xn = jnp.concatenate([xnT[0, :, half(t)], xnT[1, :, half(t)]], axis=1).astype(F32)
            m1 = jnp.mean(dxn, axis=0, keepdims=True)
            m2 = jnp.mean(dxn * xn, axis=0, keepdims=True)
            dxT = (dxn - m1 - xn * m2) * rstdT[0:1, tok]
            gob[tok, :] = (gob[tok, :].astype(F32) + dxT.T).astype(BF)

        def p4a(i, carry):
            layernorm_bwd(i, 0)
            layernorm_bwd(i, 1)
            rs = [pl.ds(pl.multiple_of((2 * i + n) * 128, 128), 128) for n in range(2)]
            full = [jnp.concatenate([qT[0, r, :], qT[1, r, :], qT[2, r, :]], axis=0) for r in rs]
            b11, b12, b21, b22 = [
                jnp.concatenate([f[:, t * T + u * HT:t * T + (u + 1) * HT] for t in range(NT)], axis=1)
                for u in range(2) for f in full]
            c11, c12, c21, c22 = _strassen(_nt, sa[5], sa[6], sa, b11, b22,
                                           _sums(b11, b12, b21, b22))
            for rows, r, dw in ((bot, rs[0], c21), (top, rs[1], c12), (top, rs[0], c11), (bot, rs[1], c22)):
                for j in range(3):
                    wf[j, rows, r] = dw[:, j * 128:(j + 1) * 128].astype(BF)
            return carry

        def unfold(g):
            r = pl.ds(pl.multiple_of(g * 128, 128), 128)
            dphi = jnp.zeros((128, 128), F32)
            for j in range(2):
                dwj = wf[j, :, r]
                dphi = dphi + _tn(w2b[j * D:(j + 1) * D, r], dwj)
                wf[j, :, r] = _nt(dwj, bd[r, :]).astype(BF)
            dphi = jnp.where(_head_mask(128, 5), dphi, 0.0)
            dphi = dphi[:, 0:32] + dphi[:, 32:64] + dphi[:, 64:96] + dphi[:, 96:128]
            wpb[r, :] = dphi.astype(BF)

        def p4b(c, carry, between=lambda i, *c: None):
            n0, n1 = halves(c)
            b11, b12, b21, b22 = [ab[:, u, :, n].reshape(HS, FC // 2) for u in range(2) for n in (n0, n1)]
            c11, c12, c21, c22 = _strassen(_nn, sa[5], sa[6], sa, b11, b22,
                                           _sums(b11, b12, b21, b22), True, between)
            for i, (rows, n, v) in enumerate(((bot, n0, c21), (top, n1, c12), (top, n0, c11), (bot, n1, c22))):
                w1b[rows, n] = v.astype(BF)
                cp(w1b.at[rows, n], dw1_h.at[rows, n], osem.at[4 + i, c]).start()
            return carry

        lax.fori_loop(0, G // 2, p4a, 0)
        o_dx.start()
        o_qkv[2].start()

        def p4u(c, carry):
            return p4b(c, carry, lambda i, *_: unfold(2 * c + i) if i < 2 else None)

        lax.fori_loop(0, G // 2, p4u, 0)
        o_qkv[0].start()
        o_qkv[1].start()
        o_phi.start()
        lax.fori_loop(G // 2, NF, p4b, 0)

    pl.run_scoped(backward_part, pltpu.VMEM((3, HD, HF), BF), pltpu.VMEM((2, D, S // 2), BF))

    o_dx.wait()
    o_dwo.wait()
    o_phi.wait()
    for c in o_qkv:
        c.wait()
    for c in range(NF):
        n0, n1 = halves(c)
        for i, (rows, n) in enumerate(((bot, n0), (top, n1), (top, n0), (bot, n1))):
            cp(w1b.at[rows, n], dw1_h.at[rows, n], osem.at[4 + i, c]).wait()


@jax.jit
def pallas_recurrent_scan__linear_kernel_hedgehog__dense_activation_relu__prompt_kernel(
    A_x: jax.Array,
    A_wqkv: jax.Array,
    A_w_phi: jax.Array,
    A_wo: jax.Array,
    B_x: jax.Array,
    B_w1: jax.Array,
    B_w2: jax.Array,
    grad_out: jax.Array,
):
    del B_x
    hbm = pl.BlockSpec(memory_space=pl.ANY)
    sds = jax.ShapeDtypeStruct
    out, dx, dwqkv, dwphi, dwo, dw1, dw2 = pl.pallas_call(
        _kernel,
        in_specs=[hbm] * 7,
        out_specs=[hbm] * 7,
        out_shape=[sds((S, D), BF), sds((S, D), BF), sds((D, 3 * D), BF), sds((D, DH), BF),
                   sds((D, D), BF), sds((D, F), BF), sds((F, D), BF)],
        scratch_shapes=[
            pltpu.VMEM((S, D), BF),
            pltpu.VMEM((S, D), BF),
            pltpu.VMEM((S, D), BF),
            pltpu.VMEM((NT, 2, T // 2, F), BF),
            pltpu.VMEM((4, D, S), BF),
            pltpu.VMEM((D, F), BF),
            pltpu.VMEM((F, D), BF),
            pltpu.VMEM((3, D, D), BF),
            pltpu.VMEM((D, D), BF),
            pltpu.VMEM((3, 5, D // 2, D // 2), BF),
            pltpu.VMEM((7, D // 2, S // 2), BF),
            pltpu.VMEM((7, S // 2, D // 2), BF),
            pltpu.VMEM((D, DH), BF),
            pltpu.VMEM((D, 128), BF),
            pltpu.VMEM((8, S), F32),
            pltpu.VMEM((P, 64, 128), F32),
            pltpu.VMEM((P, 128, 128), F32),
            pltpu.VMEM((P, 64, 128), BF),
            pltpu.VMEM((P, 128, 128), F32),
            pltpu.SemaphoreType.DMA((10,)),
            pltpu.SemaphoreType.DMA((NT,)),
            pltpu.SemaphoreType.DMA((4,)),
            pltpu.SemaphoreType.DMA((8, 8)),
        ],
        compiler_params=pltpu.CompilerParams(vmem_limit_bytes=127 * 1024 * 1024,
                                             flags={"XLA_TPU_EVENLY_DISTRIBUTE_CRITICAL_NODES": True}),
    )(A_x.reshape(S, D), A_wqkv, A_w_phi.reshape(D, DH), A_wo, B_w1, B_w2, grad_out.reshape(S, D))
    return (out.reshape(1, S, D), dx.reshape(1, S, D), dwqkv, dwphi.reshape(H, DH, DH), dwo, dw1, dw2)
```
